```python
import jax
import jax.numpy as jnp

def _softmax(x, axis=-1):
    return jax.nn.softmax(x, axis=axis)
def _gelu(x):
    return jax.nn.gelu(x, approximate=True)
def _silu(x):
    return jax.nn.silu(x)
def _sigmoid(x):
    return jax.nn.sigmoid(x)
def _layernorm(x, axis=-1, eps=1e-5):
    m = jnp.mean(x, axis=axis, keepdims=True)
    v = jnp.var(x, axis=axis, keepdims=True)
    return (x - m) / jnp.sqrt(v + eps)
def _scatter_add(tgt, idx, src, axis=0):
    return tgt.at[idx].add(src)
def _segment_sum(src, seg, n):
    return jax.ops.segment_sum(src, seg, n)
class _Rng:
    def __init__(self, key):
        self._k = key
    def _next(self):
        self._k, sub = jax.random.split(self._k)
        return sub
    def normal(self, shape):
        return jax.random.normal(self._next(), shape, dtype=jnp.bfloat16)
    def randint(self, lo, hi, shape):
        return jax.random.randint(self._next(), shape, lo, hi, dtype=jnp.int32)
    def uniform(self, shape, lo=0.0, hi=1.0):
        return jax.random.uniform(self._next(), shape, jnp.bfloat16, lo, hi)
    def permutation(self, n):
        return jax.random.permutation(self._next(), n)


kernel_name = 'gated_mix__mha_block_cached__moe_arch_mod__decode'

def setup_inputs():
    _rng = _Rng(jax.random.key(int.from_bytes(__import__("os").urandom(4), "little")))
    _w = (lambda a: (lambda t: t.astype(jnp.bfloat16) if jnp.issubdtype(t.dtype, jnp.floating) else t)(jnp.asarray(a)))
    def _A_setup():
        B, Sq, D = 4, 1, 1024
        H, Sk, Dh = 32, 8192, 128
        return {
            "x": _w((lambda *s: _rng.normal(s) * 0.05)(B, Sq, D)),
            "k_cache": _w((lambda *s: _rng.normal(s) * 0.05)(B, H, Sk, Dh)),
            "v_cache": _w((lambda *s: _rng.normal(s) * 0.05)(B, H, Sk, Dh)),
            "wq": _w((lambda *s: _rng.normal(s) * 0.05)(D, H * Dh) * (D ** -0.5)),
            "wo": _w((lambda *s: _rng.normal(s) * 0.05)(H * Dh, D) * ((H * Dh) ** -0.5)),
        }
    _A_in = _A_setup()

    def _B_setup():
        B, S, D, F, C = 4, 1, 1024, 3584, 1
        return {
            "x": _w((lambda *s: _rng.normal(s) * 0.05)(B, S, D)),
            "w_r": _w((lambda *s: _rng.normal(s) * 0.05)(D)),
            "w_gate": _w((lambda *s: _rng.normal(s) * 0.05)(D, F)),
            "w_up": _w((lambda *s: _rng.normal(s) * 0.05)(D, F)),
            "w_down": _w((lambda *s: _rng.normal(s) * 0.05)(F, D)),
        }
    _B_in = _B_setup()

    return {
        "A_x": _A_in["x"],
        "A_k_cache": _A_in["k_cache"],
        "A_v_cache": _A_in["v_cache"],
        "A_wq": _A_in["wq"],
        "A_wo": _A_in["wo"],
        "B_x": _B_in["x"],
        "B_w_r": _B_in["w_r"],
        "B_w_gate": _B_in["w_gate"],
        "B_w_up": _B_in["w_up"],
        "B_w_down": _B_in["w_down"],
        "gate_w": _w((lambda *s: _rng.normal(s) * 0.05)(1024)),
    }

def reference(A_x, A_k_cache, A_v_cache, A_wq, A_wo, B_x, B_w_r, B_w_gate, B_w_up, B_w_down, gate_w):
    def _A_ref(x, k_cache, v_cache, wq, wo):
        B, Sq, D = x.shape
        H, Dh = 32, 128
        q = (lambda x, *d: x.transpose(*d))((x @ wq).reshape(B, Sq, H, Dh), 0, 2, 1, 3)
        scores = jnp.einsum("bhqd,bhkd->bhqk", q, k_cache) * (Dh ** -0.5)
        p = _softmax(scores, axis=-1)
        o = jnp.einsum("bhqk,bhkd->bhqd", p, v_cache)
        return (lambda x, *d: x.transpose(*d))(o, 0, 2, 1, 3).reshape(B, Sq, H * Dh) @ wo

    def _B_ref(x, w_r, w_gate, w_up, w_down):
        B, S, D = x.shape
        C = 1
        r = x @ w_r
        idx = jnp.argsort(-r, axis=-1)[:, :C]
        idx_e = jnp.repeat(idx.reshape(B, C, 1), D, axis=2)
        x_sel = jnp.take_along_axis(x, idx_e, axis=1)
        g = _silu(x_sel @ w_gate)
        u = x_sel @ w_up
        y = (g * u) @ w_down
        r_sel = _sigmoid(jnp.take_along_axis(r, idx, axis=1))
        y = y * r_sel.reshape(B, C, 1)
        b_off = (jnp.arange(B) * S).reshape(B, 1)
        flat_idx = (idx + b_off).reshape(B * C)
        zero = (x * 0.0).reshape(B * S, D)
        upd = _scatter_add(zero, flat_idx, y.reshape(B * C, D), axis=0)
        return x + upd.reshape(B, S, D)

    x = A_x
    g = _sigmoid((x * gate_w).sum(-1, keepdims=True))
    a = _A_ref(x, A_k_cache, A_v_cache, A_wq, A_wo)
    b = _B_ref(x, B_w_r, B_w_gate, B_w_up, B_w_down)
    return g * a + (1 - g) * b
```

```python
import functools

import jax
import jax.numpy as jnp
import jax.experimental.pallas as pl
import jax.experimental.pallas.tpu as pltpu


def _make_kernel(B, H, SK, DH, D, F, NBUF, NWQ, FFN_ISSUE, FFN_STEP, WO_ISSUE, WO_LAG, dma_only):
    NSTEP = B * H
    scale = DH ** -0.5
    f32 = jnp.float32
    bf16 = jnp.bfloat16

    def kernel(ax_hbm, k_hbm, v_hbm, wq_hbm, wo_hbm, bx_hbm, wr_hbm, wg_hbm, wu_hbm, wd_hbm, gw_hbm,
               out_ref,
               ax_v, bx_v, wr_v, gw_v, wq_v, wo_v, wg_v, wu_v, wd_v, kbuf, vbuf, q_s, o_s, acc_s,
               sem_small, sem_wq, sem_w, sem_k, sem_v):
        small = [
            pltpu.make_async_copy(ax_hbm, ax_v, sem_small.at[0]),
            pltpu.make_async_copy(bx_hbm, bx_v, sem_small.at[1]),
            pltpu.make_async_copy(wr_hbm, wr_v, sem_small.at[2]),
            pltpu.make_async_copy(gw_hbm, gw_v, sem_small.at[3]),
        ]
        RQ = D // NWQ
        wq_cp = [pltpu.make_async_copy(wq_hbm.at[pl.ds(j * RQ, RQ)], wq_v.at[pl.ds(j * RQ, RQ)], sem_wq.at[j])
                 for j in range(NWQ)]
        wo_cp = pltpu.make_async_copy(wo_hbm, wo_v, sem_w.at[0])
        wg_cp = pltpu.make_async_copy(wg_hbm, wg_v, sem_w.at[1])
        wu_cp = pltpu.make_async_copy(wu_hbm, wu_v, sem_w.at[2])
        wd_cp = pltpu.make_async_copy(wd_hbm, wd_v, sem_w.at[3])

        def k_cp(i):
            slot = i % NBUF
            return pltpu.make_async_copy(k_hbm.at[i % B, i // B], kbuf.at[slot], sem_k.at[slot])

        def v_cp(i):
            slot = i % NBUF
            return pltpu.make_async_copy(v_hbm.at[i % B, i // B], vbuf.at[slot], sem_v.at[slot])

        for c in small:
            c.start()
        for c in wq_cp:
            c.start()
        for i in range(NBUF - 1):
            k_cp(i).start()
            v_cp(i).start()

        row = jax.lax.broadcasted_iota(jnp.int32, (8, D), 0)

        def rows8(ref):
            out = jnp.zeros((8, D), f32)
            for b in range(B):
                out = jnp.where(row == b, jnp.broadcast_to(ref[b].astype(f32), (8, D)), out)
            return out

        for c in small:
            c.wait()
        xa = rows8(ax_v).astype(bf16)
        q = jnp.zeros((8, H * DH), f32)
        for j in range(NWQ):
            wq_cp[j].wait()
            q = q + jnp.dot(xa[:, j * RQ:(j + 1) * RQ], wq_v[pl.ds(j * RQ, RQ), :], preferred_element_type=f32)
        qb = q.astype(bf16)
        for h in range(H):
            q_s[h] = qb[:, h * DH:(h + 1) * DH]
        acc_s[...] = jnp.zeros_like(acc_s)

        def out_proj(h):
            acc_s[...] += jnp.dot(o_s[h].astype(bf16),
                                  wo_v[pl.ds(pl.multiple_of(h * DH, DH), DH), :],
                                  preferred_element_type=f32)

        def step(i, carry):
            h = i // B
            b = i % B
            slot = i % NBUF

            @pl.when(i + NBUF - 1 < NSTEP)
            def _():
                k_cp(i + NBUF - 1).start()
                v_cp(i + NBUF - 1).start()

            @pl.when(i == WO_ISSUE)
            def _():
                wo_cp.start()

            @pl.when(i == FFN_ISSUE)
            def _():
                wg_cp.start()

            @pl.when(i == FFN_ISSUE + 2)
            def _():
                wu_cp.start()

            @pl.when(i == FFN_ISSUE + 4)
            def _():
                wd_cp.start()

            k_cp(i).wait()
            if not dma_only:
                s = jax.lax.dot_general(q_s[h], kbuf[slot], (((1,), (1,)), ((), ())),
                                        preferred_element_type=f32) * scale
                m = jnp.max(s, axis=-1, keepdims=True)
                p = jnp.exp(s - m)
                l = jnp.sum(p, axis=-1, keepdims=True)
            v_cp(i).wait()
            if not dma_only:
                o = jnp.dot(p.astype(bf16), vbuf[slot], preferred_element_type=f32) / l
                r8 = jax.lax.broadcasted_iota(jnp.int32, (8, DH), 0)

                @pl.when(b == 0)
                def _():
                    o_s[h] = o

                @pl.when(b != 0)
                def _():
                    o_s[h] = jnp.where(r8 == b, o, o_s[h])
            else:
                o_s[h] = jnp.zeros((8, DH), f32)

            @pl.when(i == WO_LAG * B + B - 1)
            def _():
                wo_cp.wait()

            @pl.when(jnp.logical_and(b == B - 1, h >= WO_LAG))
            def _():
                out_proj(h - WO_LAG)

            @pl.when(i == FFN_STEP)
            def _():
                wg_cp.wait()
                wu_cp.wait()
                wd_cp.wait()
                xb = rows8(ax_v)
                xbb = xb.astype(bf16)
                g = jnp.dot(xbb, wg_v[...], preferred_element_type=f32)
                u = jnp.dot(xbb, wu_v[...], preferred_element_type=f32)
                hdn = (g * jax.nn.sigmoid(g)) * u
                y = jnp.dot(hdn.astype(bf16), wd_v[...], preferred_element_type=f32)
                r = jnp.sum(xb * wr_v[...].astype(f32).reshape(1, D), axis=-1, keepdims=True)
                bout = xb + (xb * 0.0 + y * jax.nn.sigmoid(r))
                ga = jax.nn.sigmoid(jnp.sum(rows8(ax_v) * gw_v[...].astype(f32).reshape(1, D),
                                            axis=-1, keepdims=True))
                res_s[...] = (1.0 - ga) * bout
            return carry

        def body(res_s_):
            nonlocal res_s
            res_s = res_s_
            jax.lax.fori_loop(0, NSTEP, step, 0)
            for h in range(H - WO_LAG, H):
                out_proj(h)
            ga = jax.nn.sigmoid(jnp.sum(rows8(ax_v) * gw_v[...].astype(f32).reshape(1, D),
                                        axis=-1, keepdims=True))
            res = (ga * acc_s[...] + res_s[...]).astype(out_ref.dtype)
            for b in range(B):
                out_ref[b] = res[b:b + 1, :]

        res_s = None
        pl.run_scoped(body, pltpu.VMEM((8, D), f32))

    return kernel


def _impl(A_x, A_k_cache, A_v_cache, A_wq, A_wo, B_x, B_w_r, B_w_gate, B_w_up, B_w_down, gate_w,
          NBUF=8, NWQ=8, FFN_ISSUE=12, FFN_STEP=40, WO_ISSUE=1, WO_LAG=3, dma_only=False):
    B, H, SK, DH = A_k_cache.shape
    D = A_x.shape[-1]
    F = B_w_gate.shape[-1]
    bf16 = jnp.bfloat16
    kernel = _make_kernel(B, H, SK, DH, D, F, NBUF, NWQ, FFN_ISSUE, FFN_STEP, WO_ISSUE, WO_LAG, dma_only)
    any_spec = pl.BlockSpec(memory_space=pl.ANY)
    return pl.pallas_call(
        kernel,
        out_shape=jax.ShapeDtypeStruct(A_x.shape, A_x.dtype),
        in_specs=[any_spec] * 11,
        out_specs=pl.BlockSpec(memory_space=pltpu.VMEM),
        scratch_shapes=[
            pltpu.VMEM(A_x.shape, A_x.dtype),
            pltpu.VMEM(B_x.shape, B_x.dtype),
            pltpu.VMEM(B_w_r.shape, B_w_r.dtype),
            pltpu.VMEM(gate_w.shape, gate_w.dtype),
            pltpu.VMEM(A_wq.shape, A_wq.dtype),
            pltpu.VMEM(A_wo.shape, A_wo.dtype),
            pltpu.VMEM(B_w_gate.shape, B_w_gate.dtype),
            pltpu.VMEM(B_w_up.shape, B_w_up.dtype),
            pltpu.VMEM(B_w_down.shape, B_w_down.dtype),
            pltpu.VMEM((NBUF, SK, DH), A_k_cache.dtype),
            pltpu.VMEM((NBUF, SK, DH), A_v_cache.dtype),
            pltpu.VMEM((H, 8, DH), bf16),
            pltpu.VMEM((H, 8, DH), jnp.float32),
            pltpu.VMEM((8, D), jnp.float32),
            pltpu.SemaphoreType.DMA((4,)),
            pltpu.SemaphoreType.DMA((NWQ,)),
            pltpu.SemaphoreType.DMA((4,)),
            pltpu.SemaphoreType.DMA((NBUF,)),
            pltpu.SemaphoreType.DMA((NBUF,)),
        ],
        compiler_params=pltpu.CompilerParams(vmem_limit_bytes=110 * 1024 * 1024),
    )(A_x, A_k_cache, A_v_cache, A_wq, A_wo, B_x, B_w_r, B_w_gate, B_w_up, B_w_down, gate_w)


@jax.jit
def pallas_gated_mix__mha_block_cached__moe_arch_mod__decode_kernel(
    A_x: jax.Array,
    A_k_cache: jax.Array,
    A_v_cache: jax.Array,
    A_wq: jax.Array,
    A_wo: jax.Array,
    B_x: jax.Array,
    B_w_r: jax.Array,
    B_w_gate: jax.Array,
    B_w_up: jax.Array,
    B_w_down: jax.Array,
    gate_w: jax.Array,
):
    return _impl(A_x, A_k_cache, A_v_cache, A_wq, A_wo, B_x, B_w_r, B_w_gate, B_w_up, B_w_down, gate_w)
```

```python
import jax
import jax.numpy as jnp
from jax import lax
import jax.experimental.pallas as pl
import jax.experimental.pallas.tpu as pltpu


def _chunks(total, rows, ways):
    cs = [(o, min(rows, total - o)) for o in range(0, total, rows)]
    per = -(-len(cs) // ways)
    return [cs[s * per + u] for u in range(per) for s in range(ways) if s * per + u < len(cs)]


def _merge(*lists):
    ev = [((i + 0.5) / len(l), a, e) for a, l in enumerate(lists) for i, e in enumerate(l)]
    return [(a, e) for _, a, e in sorted(ev, key=lambda t: t[:2])]


def _make_kernel(B, H, SK, DH, D, F, NBUF, KCH, VCH, dma_only):
    NSTEP = B * H
    WSTEPS = 32
    FFN_STEP = WSTEPS + NBUF + 1
    WO_HEAD = FFN_STEP // B + 2
    scale = DH ** -0.5
    f32, bf16 = jnp.float32, jnp.bfloat16
    kv_order = _merge(_chunks(SK, *KCH), _chunks(SK, *VCH))
    CB = 512
    RQ, RO, RG, RD = D // 2 // WSTEPS, H * DH // WSTEPS, D // WSTEPS, F // WSTEPS

    def kernel(ax_hbm, k_hbm, v_hbm, wq_hbm, wo_hbm, wr_hbm, wg_hbm, wu_hbm, wd_hbm, gw_hbm,
               out_ref,
               ax_v, wr_v, gw_v, wq_v, wo_v, wg_v, wu_v, wd_v, kbuf, vbuf, q_s, o_s, acc_s, res_s,
               sem_small, sem_w, sem_k, sem_v):
        def copy(src, dst, sem, idx, queue):
            pltpu.make_async_copy(src.at[idx], dst.at[idx], sem).start(priority=queue)

        def wait_all(dst, sem):
            pltpu.make_async_copy(dst, dst, sem).wait()

        def start_kv(i):
            b, h, slot = i % B, i // B, i % NBUF
            for a, (o, r) in kv_order:
                src, dst, sem = ((k_hbm, kbuf, sem_k), (v_hbm, vbuf, sem_v))[a]
                pltpu.make_async_copy(src.at[b, h, pl.ds(o, r)], dst.at[slot, pl.ds(o, r)],
                                      sem.at[slot]).start(priority=a)

        def start_weights(i):
            def tiles(rows, cols):
                r0 = pl.multiple_of(i * rows, rows)
                cb = CB * 32 // rows if rows <= 32 else None
                if cb is not None:
                    return [(pl.ds(r0, rows), pl.ds(c, cb)) for c in range(0, cols, cb)]
                return [(pl.ds(pl.multiple_of(r0 + r, 16), 16), slice(None)) for r in range(0, rows, 16)]
            q0 = [(wo_hbm, wo_v, sem_w.at[2], t) for t in tiles(RO, D)] + \
                 [(wg_hbm, wg_v, sem_w.at[4], t) for t in tiles(RG, F)]
            q1 = [(wd_hbm, wd_v, sem_w.at[3], t) for t in tiles(RD, D)] + \
                 [(wu_hbm, wu_v, sem_w.at[5], t) for t in tiles(RG, F)]
            for a, (src, dst, sem, t) in _merge(q0, q1):
                copy(src, dst, sem, t, a)

        small = [pltpu.make_async_copy(s, d, sem_small.at[j])
                 for j, (s, d) in enumerate(((ax_hbm, ax_v), (wr_hbm, wr_v), (gw_hbm, gw_v)))]
        for c in small:
            c.start()

        @pl.loop(0, WSTEPS)
        def _(i):
            for c in range(0, H * DH, 2 * CB):
                for a in range(2):
                    r0 = pl.multiple_of(a * (D // 2) + i * RQ, RQ)
                    copy(wq_hbm, wq_v, sem_w.at[a], (pl.ds(r0, RQ), pl.ds(c, 2 * CB)), a)

        @pl.loop(0, NBUF - 1)
        def _(i):
            start_kv(i)

        for c in small:
            c.wait()
        x = ax_v[...].astype(f32)
        x8 = jnp.concatenate([x, jnp.zeros((8 - B, D), f32)], axis=0)
        xb = x8.astype(bf16)
        gate = jax.nn.sigmoid(jnp.sum(x8 * gw_v[...].astype(f32).reshape(1, D), axis=-1, keepdims=True))
        for a in range(2):
            wait_all(wq_v.at[pl.ds(a * (D // 2), D // 2)], sem_w.at[a])
        qb = jnp.dot(xb, wq_v[...], preferred_element_type=f32).astype(bf16)
        for h in range(H):
            q_s[h] = qb[:, h * DH:(h + 1) * DH]
        acc_s[...] = jnp.zeros_like(acc_s)

        def out_proj(h):
            acc_s[...] += jnp.dot(o_s[h].astype(bf16), wo_v[pl.ds(pl.multiple_of(h * DH, DH), DH), :],
                                  preferred_element_type=f32)

        @pl.loop(0, NSTEP)
        def _(i):
            h, b, slot = i // B, i % B, i % NBUF

            @pl.when(i + NBUF - 1 < NSTEP)
            def _():
                start_kv(i + NBUF - 1)

            @pl.when(i < WSTEPS)
            def _():
                start_weights(i)

            wait_all(kbuf.at[slot], sem_k.at[slot])
            if not dma_only:
                s = lax.dot_general(q_s[h], kbuf[slot], (((1,), (1,)), ((), ())),
                                    preferred_element_type=f32) * scale
                m = jnp.max(s, axis=-1, keepdims=True)
                p = jnp.exp(s - m)
                l = jnp.sum(p, axis=-1, keepdims=True)
            wait_all(vbuf.at[slot], sem_v.at[slot])
            if not dma_only:
                o = jnp.dot(p.astype(bf16), vbuf[slot], preferred_element_type=f32) / l
            else:
                o = jnp.zeros((8, DH), f32)

            @pl.when(b == 0)
            def _():
                o_s[h] = o

            @pl.when(b != 0)
            def _():
                o_s[h] = jnp.where(lax.broadcasted_iota(jnp.int32, (8, DH), 0) == b, o, o_s[h])

            @pl.when(i == WO_HEAD * B)
            def _():
                wait_all(wo_v, sem_w.at[2])

                @pl.loop(0, WO_HEAD)
                def _(hh):
                    out_proj(hh)

            @pl.when(jnp.logical_and(b == B - 1, h >= WO_HEAD))
            def _():
                out_proj(h)

            @pl.when(i == FFN_STEP)
            def _():
                wait_all(wd_v, sem_w.at[3])
                wait_all(wg_v, sem_w.at[4])
                wait_all(wu_v, sem_w.at[5])
                g = jnp.dot(xb, wg_v[...], preferred_element_type=f32)
                u = jnp.dot(xb, wu_v[...], preferred_element_type=f32)
                y = jnp.dot(((g * jax.nn.sigmoid(g)) * u).astype(bf16), wd_v[...], preferred_element_type=f32)
                r = jnp.sum(x8 * wr_v[...].astype(f32).reshape(1, D), axis=-1, keepdims=True)
                res_s[...] = (1.0 - gate) * (x8 + (x8 * 0.0 + y * jax.nn.sigmoid(r)))

        out_ref[...] = (gate * acc_s[...] + res_s[...])[:B].astype(out_ref.dtype)

    return kernel


def _impl(A_x, A_k_cache, A_v_cache, A_wq, A_wo, B_x, B_w_r, B_w_gate, B_w_up, B_w_down, gate_w,
          NBUF=4, KCH=(96, 4), VCH=(80, 4), dma_only=False):
    del B_x
    B, H, SK, DH = A_k_cache.shape
    D = A_x.shape[-1]
    F = B_w_gate.shape[-1]
    x2 = A_x.reshape(B, D)
    vmem = lambda a: pltpu.VMEM(a.shape, a.dtype)
    out = pl.pallas_call(
        _make_kernel(B, H, SK, DH, D, F, NBUF, KCH, VCH, dma_only),
        out_shape=jax.ShapeDtypeStruct((B, D), A_x.dtype),
        in_specs=[pl.BlockSpec(memory_space=pl.ANY)] * 10,
        out_specs=pl.BlockSpec(memory_space=pltpu.VMEM),
        scratch_shapes=[
            vmem(x2), vmem(B_w_r), vmem(gate_w),
            vmem(A_wq), vmem(A_wo), vmem(B_w_gate), vmem(B_w_up), vmem(B_w_down),
            pltpu.VMEM((NBUF, SK, DH), A_k_cache.dtype),
            pltpu.VMEM((NBUF, SK, DH), A_v_cache.dtype),
            pltpu.VMEM((H, 8, DH), jnp.bfloat16),
            pltpu.VMEM((H, 8, DH), jnp.float32),
            pltpu.VMEM((8, D), jnp.float32),
            pltpu.VMEM((8, D), jnp.float32),
            pltpu.SemaphoreType.DMA((3,)),
            pltpu.SemaphoreType.DMA((6,)),
            pltpu.SemaphoreType.DMA((NBUF,)),
            pltpu.SemaphoreType.DMA((NBUF,)),
        ],
        compiler_params=pltpu.CompilerParams(vmem_limit_bytes=100 * 1024 * 1024),
    )(x2, A_k_cache, A_v_cache, A_wq, A_wo, B_w_r, B_w_gate, B_w_up, B_w_down, gate_w)
    return out.reshape(A_x.shape)


@jax.jit
def pallas_gated_mix__mha_block_cached__moe_arch_mod__decode_kernel(
    A_x: jax.Array,
    A_k_cache: jax.Array,
    A_v_cache: jax.Array,
    A_wq: jax.Array,
    A_wo: jax.Array,
    B_x: jax.Array,
    B_w_r: jax.Array,
    B_w_gate: jax.Array,
    B_w_up: jax.Array,
    B_w_down: jax.Array,
    gate_w: jax.Array,
):
    return _impl(A_x, A_k_cache, A_v_cache, A_wq, A_wo, B_x, B_w_r, B_w_gate, B_w_up, B_w_down, gate_w)
```

```python
import jax
import jax.numpy as jnp
from jax import lax
import jax.experimental.pallas as pl
import jax.experimental.pallas.tpu as pltpu


def _chunks(total, rows, ways):
    cs = [(o, min(rows, total - o)) for o in range(0, total, rows)]
    per = -(-len(cs) // ways)
    return [cs[s * per + u] for u in range(per) for s in range(ways) if s * per + u < len(cs)]


def _merge(*lists):
    ev = [((i + 0.5) / len(l), a, e) for a, l in enumerate(lists) for i, e in enumerate(l)]
    return [(a, e) for _, a, e in sorted(ev, key=lambda t: t[:2])]


def _make_kernel(B, H, SK, DH, D, F, NBUF, KCH, VCH, WT, QT, dma_only):
    NSTEP = B * H
    WSTEPS = 32
    FFN_STEP = WSTEPS + NBUF + 1
    WO_HEAD = FFN_STEP // B + 2
    scale = DH ** -0.5
    f32, bf16 = jnp.float32, jnp.bfloat16
    kv_order = _merge(_chunks(SK, *KCH), _chunks(SK, *VCH))
    QSTEPS = 8

    def kernel(ax_hbm, k_hbm, v_hbm, wq_hbm, wo_hbm, wr_hbm, wg_hbm, wu_hbm, wd_hbm, gw_hbm,
               out_ref,
               ax_v, wr_v, gw_v, wq_v, wo_v, wg_v, wu_v, wd_v, kbuf, vbuf, q_s, o_s, acc_s, res_s,
               sem_small, sem_w, sem_k, sem_v, sem_x):
        def copy(src, dst, sem, idx, queue):
            pltpu.make_async_copy(src.at[idx], dst.at[idx], sem).start(priority=queue)

        def wait_all(dst, sem):
            pltpu.make_async_copy(dst, dst, sem).wait()

        def start_kv(i):
            b, h, slot = i % B, i // B, i % NBUF
            for a, (o, r) in kv_order:
                src, dst, sem = ((k_hbm, kbuf, sem_k), (v_hbm, vbuf, sem_v))[a]
                pltpu.make_async_copy(src.at[b, h, pl.ds(o, r)], dst.at[slot, pl.ds(o, r)],
                                      sem.at[slot]).start(priority=a)

        def start_kv_last():
            i, half = NSTEP - 1, SK // 2
            for t, (src, dst, sem) in enumerate(((k_hbm, kbuf, sem_k), (v_hbm, vbuf, sem_v))):
                for o, r in _chunks(half, *KCH):
                    for a in range(2):
                        pltpu.make_async_copy(src.at[i % B, i // B, pl.ds(a * half + o, r)],
                                              dst.at[i % NBUF, pl.ds(a * half + o, r)],
                                              sem_x.at[t] if a else sem.at[i % NBUF]).start(priority=a)

        def wait_kv(i, t):
            buf, sem = ((kbuf, sem_k), (vbuf, sem_v))[t]
            slot, half = i % NBUF, SK // 2
            wait_all(buf.at[slot, pl.ds(0, half)], sem.at[slot])

            @pl.when(i < NSTEP - 1)
            def _():
                wait_all(buf.at[slot, pl.ds(half, half)], sem.at[slot])

            @pl.when(i == NSTEP - 1)
            def _():
                wait_all(buf.at[slot, pl.ds(half, half)], sem_x.at[t])

        def tiles(i, steps, shape, tr, tc, ways=4):
            rows = shape[0] // steps // ways
            return [(pl.ds(pl.multiple_of(w * (shape[0] // ways) + i * rows + r, 8), tr), pl.ds(c, tc))
                    for r in range(0, rows, tr) for c in range(0, shape[1], tc) for w in range(ways)]

        def start_weights(i):
            q0 = [(wg_hbm, wg_v, sem_w.at[4], t) for t in tiles(i, WSTEPS, (D, F), WT[0], WT[1])]
            q1 = [(wu_hbm, wu_v, sem_w.at[5], t) for t in tiles(i, WSTEPS, (D, F), WT[0], WT[1])]
            for a, (src, dst, sem, t) in _merge(q0, q1):
                copy(src, dst, sem, t, a)
            q0 = tiles(i, WSTEPS, (H * DH, D), WT[2], D)
            q1 = tiles(i, F // 128, (F, D), WT[2], D)

            @pl.when(i < F // 128)
            def _():
                for t0, t1 in zip(q0, q1):
                    copy(wo_hbm, wo_v, sem_w.at[2], t0, 0)
                    copy(wd_hbm, wd_v, sem_w.at[3], t1, 1)

            @pl.when(i >= F // 128)
            def _():
                for t0 in q0:
                    copy(wo_hbm, wo_v, sem_w.at[2], t0, 0)

        small = [pltpu.make_async_copy(s, d, sem_small.at[j])
                 for j, (s, d) in enumerate(((ax_hbm, ax_v), (wr_hbm, wr_v), (gw_hbm, gw_v)))]
        for c in small:
            c.start()

        @pl.loop(0, QSTEPS)
        def _(i):
            for rs, cs in tiles(i, QSTEPS, (D // 2, H * DH), QT[0], QT[1], QT[2]):
                for a in range(2):
                    r0 = pl.multiple_of(a * (D // 2) + rs.start, 8)
                    copy(wq_hbm, wq_v, sem_w.at[a], (pl.ds(r0, QT[0]), cs), a)

        @pl.loop(0, NBUF - 1)
        def _(i):
            start_kv(i)

        for c in small:
            c.wait()
        x = ax_v[...].astype(f32)
        x8 = jnp.concatenate([x, jnp.zeros((8 - B, D), f32)], axis=0)
        xb = x8.astype(bf16)
        gate = jax.nn.sigmoid(jnp.sum(x8 * gw_v[...].astype(f32).reshape(1, D), axis=-1, keepdims=True))
        for a in range(2):
            wait_all(wq_v.at[pl.ds(a * (D // 2), D // 2)], sem_w.at[a])
        qb = jnp.dot(xb, wq_v[...], preferred_element_type=f32).astype(bf16)
        for h in range(H):
            q_s[h] = qb[:, h * DH:(h + 1) * DH]
        acc_s[...] = jnp.zeros_like(acc_s)

        def out_proj(h):
            acc_s[...] += jnp.dot(o_s[h].astype(bf16), wo_v[pl.ds(pl.multiple_of(h * DH, DH), DH), :],
                                  preferred_element_type=f32)

        @pl.loop(0, NSTEP)
        def _(i):
            h, b, slot = i // B, i % B, i % NBUF

            @pl.when(i + NBUF < NSTEP)
            def _():
                start_kv(i + NBUF - 1)

            @pl.when(i + NBUF == NSTEP)
            def _():
                start_kv_last()

            @pl.when(i < WSTEPS)
            def _():
                start_weights(i)

            wait_kv(i, 0)
            if not dma_only:
                s = lax.dot_general(q_s[h], kbuf[slot], (((1,), (1,)), ((), ())),
                                    preferred_element_type=f32) * scale
                m = jnp.max(s, axis=-1, keepdims=True)
                p = jnp.exp(s - m)
                l = jnp.sum(p, axis=-1, keepdims=True)
            wait_kv(i, 1)
            if not dma_only:
                o = jnp.dot(p.astype(bf16), vbuf[slot], preferred_element_type=f32) / l
            else:
                o = jnp.zeros((8, DH), f32)

            @pl.when(b == 0)
            def _():
                o_s[h] = o

            @pl.when(b != 0)
            def _():
                o_s[h] = jnp.where(lax.broadcasted_iota(jnp.int32, (8, DH), 0) == b, o, o_s[h])

            @pl.when(i == WO_HEAD * B)
            def _():
                wait_all(wo_v, sem_w.at[2])

                @pl.loop(0, WO_HEAD)
                def _(hh):
                    out_proj(hh)

            @pl.when(jnp.logical_and(b == B - 1, h >= WO_HEAD))
            def _():
                out_proj(h)

            @pl.when(i == FFN_STEP)
            def _():
                wait_all(wd_v, sem_w.at[3])
                wait_all(wg_v, sem_w.at[4])
                wait_all(wu_v, sem_w.at[5])
                g = jnp.dot(xb, wg_v[...], preferred_element_type=f32)
                u = jnp.dot(xb, wu_v[...], preferred_element_type=f32)
                y = jnp.dot(((g * jax.nn.sigmoid(g)) * u).astype(bf16), wd_v[...], preferred_element_type=f32)
                r = jnp.sum(x8 * wr_v[...].astype(f32).reshape(1, D), axis=-1, keepdims=True)
                res_s[...] = (1.0 - gate) * (x8 + (x8 * 0.0 + y * jax.nn.sigmoid(r)))

        out_ref[...] = (gate * acc_s[...] + res_s[...])[:B].astype(out_ref.dtype)

    return kernel


def _impl(A_x, A_k_cache, A_v_cache, A_wq, A_wo, B_x, B_w_r, B_w_gate, B_w_up, B_w_down, gate_w,
          NBUF=2, KCH=(160, 4), VCH=(160, 4), WT=(8, 1792, 16), QT=(8, 2048, 4), dma_only=False):
    del B_x
    B, H, SK, DH = A_k_cache.shape
    D = A_x.shape[-1]
    F = B_w_gate.shape[-1]
    x2 = A_x.reshape(B, D)
    vmem = lambda a: pltpu.VMEM(a.shape, a.dtype)
    out = pl.pallas_call(
        _make_kernel(B, H, SK, DH, D, F, NBUF, KCH, VCH, WT, QT, dma_only),
        out_shape=jax.ShapeDtypeStruct((B, D), A_x.dtype),
        in_specs=[pl.BlockSpec(memory_space=pl.ANY)] * 10,
        out_specs=pl.BlockSpec(memory_space=pltpu.VMEM),
        scratch_shapes=[
            vmem(x2), vmem(B_w_r), vmem(gate_w),
            vmem(A_wq), vmem(A_wo), vmem(B_w_gate), vmem(B_w_up), vmem(B_w_down),
            pltpu.VMEM((NBUF, SK, DH), A_k_cache.dtype),
            pltpu.VMEM((NBUF, SK, DH), A_v_cache.dtype),
            pltpu.VMEM((H, 8, DH), jnp.bfloat16),
            pltpu.VMEM((H, 8, DH), jnp.float32),
            pltpu.VMEM((8, D), jnp.float32),
            pltpu.VMEM((8, D), jnp.float32),
            pltpu.SemaphoreType.DMA((3,)),
            pltpu.SemaphoreType.DMA((6,)),
            pltpu.SemaphoreType.DMA((NBUF,)),
            pltpu.SemaphoreType.DMA((NBUF,)),
            pltpu.SemaphoreType.DMA((2,)),
        ],
        compiler_params=pltpu.CompilerParams(vmem_limit_bytes=100 * 1024 * 1024, disable_bounds_checks=True),
    )(x2, A_k_cache, A_v_cache, A_wq, A_wo, B_w_r, B_w_gate, B_w_up, B_w_down, gate_w)
    return out.reshape(A_x.shape)


@jax.jit
def pallas_gated_mix__mha_block_cached__moe_arch_mod__decode_kernel(
    A_x: jax.Array,
    A_k_cache: jax.Array,
    A_v_cache: jax.Array,
    A_wq: jax.Array,
    A_wo: jax.Array,
    B_x: jax.Array,
    B_w_r: jax.Array,
    B_w_gate: jax.Array,
    B_w_up: jax.Array,
    B_w_down: jax.Array,
    gate_w: jax.Array,
):
    return _impl(A_x, A_k_cache, A_v_cache, A_wq, A_wo, B_x, B_w_r, B_w_gate, B_w_up, B_w_down, gate_w)
```

```python
import jax
import jax.numpy as jnp
from jax import lax
import jax.experimental.pallas as pl
import jax.experimental.pallas.tpu as pltpu


def _chunks(total, rows, ways):
    cs = [(o, min(rows, total - o)) for o in range(0, total, rows)]
    per = -(-len(cs) // ways)
    return [cs[s * per + u] for u in range(per) for s in range(ways) if s * per + u < len(cs)]


def _merge(*lists):
    ev = [((i + 0.5) / len(l), a, e) for a, l in enumerate(lists) for i, e in enumerate(l)]
    return [(a, e) for _, a, e in sorted(ev, key=lambda t: t[:2])]


def _make_kernel(B, H, SK, DH, D, F, NBUF, KCH, VCH, WT, QT):
    NSTEP = B * H
    WSTEPS = 32
    FFN_STEP = WSTEPS + NBUF + 1
    WO_HEAD = FFN_STEP // B + 2
    scale = DH ** -0.5
    f32, bf16 = jnp.float32, jnp.bfloat16
    kv_order = _merge(_chunks(SK, *KCH), _chunks(SK, *VCH))
    QSTEPS = 8

    def kernel(ax_hbm, k_hbm, v_hbm, wq_hbm, wo_hbm, wr_hbm, wg_hbm, wu_hbm, wd_hbm, gw_hbm,
               out_ref,
               ax_v, wr_v, gw_v, wq_v, wo_v, wg_v, wu_v, wd_v, kbuf, vbuf, q_s, o_s, acc_s, res_s,
               sem_small, sem_w, sem_k, sem_v, sem_x):
        def copy(src, dst, sem, idx, queue):
            pltpu.make_async_copy(src.at[idx], dst.at[idx], sem).start(priority=queue)

        def wait_all(dst, sem):
            pltpu.make_async_copy(dst, dst, sem).wait()

        def start_kv(i):
            b, h, slot = i % B, i // B, i % NBUF
            for a, (o, r) in kv_order:
                src, dst, sem = ((k_hbm, kbuf, sem_k), (v_hbm, vbuf, sem_v))[a]
                pltpu.make_async_copy(src.at[b, h, pl.ds(o, r)], dst.at[slot, pl.ds(o, r)],
                                      sem.at[slot]).start(priority=a)

        def start_kv_last():
            i, half = NSTEP - 1, SK // 2
            for t, (src, dst, sem) in enumerate(((k_hbm, kbuf, sem_k), (v_hbm, vbuf, sem_v))):
                for o, r in _chunks(half, *KCH):
                    for a in range(2):
                        pltpu.make_async_copy(src.at[i % B, i // B, pl.ds(a * half + o, r)],
                                              dst.at[i % NBUF, pl.ds(a * half + o, r)],
                                              sem_x.at[t] if a else sem.at[i % NBUF]).start(priority=a)

        def wait_kv(i, t):
            buf, sem = ((kbuf, sem_k), (vbuf, sem_v))[t]
            slot, half = i % NBUF, SK // 2
            wait_all(buf.at[slot, pl.ds(0, half)], sem.at[slot])

            @pl.when(i < NSTEP - 1)
            def _():
                wait_all(buf.at[slot, pl.ds(half, half)], sem.at[slot])

            @pl.when(i == NSTEP - 1)
            def _():
                wait_all(buf.at[slot, pl.ds(half, half)], sem_x.at[t])

        def tiles(i, steps, shape, tr, tc, ways=4):
            rows = shape[0] // steps // ways
            return [(pl.ds(pl.multiple_of(w * (shape[0] // ways) + i * rows + r, 8), tr), pl.ds(c, tc))
                    for r in range(0, rows, tr) for c in range(0, shape[1], tc) for w in range(ways)]

        def start_weights(i):
            q0 = [(wg_hbm, wg_v, sem_w.at[4], t) for t in tiles(i, WSTEPS, (D, F), WT[0], WT[1])]
            q1 = [(wu_hbm, wu_v, sem_w.at[5], t) for t in tiles(i, WSTEPS, (D, F), WT[0], WT[1])]
            for a, (src, dst, sem, t) in _merge(q0, q1):
                copy(src, dst, sem, t, a)
            q0 = tiles(i, WSTEPS, (H * DH, D), WT[2], D)
            q1 = tiles(i, F // 128, (F, D), WT[2], D)

            @pl.when(i < F // 128)
            def _():
                for t0, t1 in zip(q0, q1):
                    copy(wo_hbm, wo_v, sem_w.at[2], t0, 0)
                    copy(wd_hbm, wd_v, sem_w.at[3], t1, 1)

            @pl.when(i >= F // 128)
            def _():
                for t0 in q0:
                    copy(wo_hbm, wo_v, sem_w.at[2], t0, 0)

        small = [pltpu.make_async_copy(s, d, sem_small.at[j])
                 for j, (s, d) in enumerate(((ax_hbm, ax_v), (wr_hbm, wr_v), (gw_hbm, gw_v)))]
        for c in small:
            c.start()

        @pl.loop(0, QSTEPS)
        def _(i):
            for rs, cs in tiles(i, QSTEPS, (D // 2, H * DH), QT[0], QT[1], QT[2]):
                for a in range(2):
                    r0 = pl.multiple_of(a * (D // 2) + rs.start, 8)
                    copy(wq_hbm, wq_v, sem_w.at[a], (pl.ds(r0, QT[0]), cs), a)

        @pl.loop(0, NBUF - 1)
        def _(i):
            start_kv(i)

        for c in small:
            c.wait()
        x = ax_v[...].astype(f32)
        x8 = jnp.concatenate([x, jnp.zeros((8 - B, D), f32)], axis=0)
        xb = x8.astype(bf16)
        gate = jax.nn.sigmoid(jnp.sum(x8 * gw_v[...].astype(f32).reshape(1, D), axis=-1, keepdims=True))
        for a in range(2):
            wait_all(wq_v.at[pl.ds(a * (D // 2), D // 2)], sem_w.at[a])
        qb = jnp.dot(xb, wq_v[...], preferred_element_type=f32).astype(bf16)
        for h in range(H):
            q_s[h] = qb[:, h * DH:(h + 1) * DH]
        acc_s[...] = jnp.zeros_like(acc_s)

        def out_proj(h):
            acc_s[...] += jnp.dot(o_s[h].astype(bf16), wo_v[pl.ds(pl.multiple_of(h * DH, DH), DH), :],
                                  preferred_element_type=f32)

        @pl.loop(0, NSTEP)
        def _(i):
            h, b, slot = i // B, i % B, i % NBUF

            @pl.when(i + NBUF < NSTEP)
            def _():
                start_kv(i + NBUF - 1)

            @pl.when(i + NBUF == NSTEP)
            def _():
                start_kv_last()

            @pl.when(i < WSTEPS)
            def _():
                start_weights(i)

            wait_kv(i, 0)
            s = lax.dot_general(q_s[h], kbuf[slot], (((1,), (1,)), ((), ())),
                                preferred_element_type=f32) * scale
            m = jnp.max(s, axis=-1, keepdims=True)
            p = jnp.exp(s - m)
            l = jnp.sum(p, axis=-1, keepdims=True)
            wait_kv(i, 1)
            o = jnp.dot(p.astype(bf16), vbuf[slot], preferred_element_type=f32) / l

            @pl.when(b == 0)
            def _():
                o_s[h] = o

            @pl.when(b != 0)
            def _():
                o_s[h] = jnp.where(lax.broadcasted_iota(jnp.int32, (8, DH), 0) == b, o, o_s[h])

            @pl.when(i == WO_HEAD * B)
            def _():
                wait_all(wo_v, sem_w.at[2])

                @pl.loop(0, WO_HEAD)
                def _(hh):
                    out_proj(hh)

            @pl.when(jnp.logical_and(b == B - 1, h >= WO_HEAD))
            def _():
                out_proj(h)

            @pl.when(i == FFN_STEP)
            def _():
                wait_all(wd_v, sem_w.at[3])
                wait_all(wg_v, sem_w.at[4])
                wait_all(wu_v, sem_w.at[5])
                g = jnp.dot(xb, wg_v[...], preferred_element_type=f32)
                u = jnp.dot(xb, wu_v[...], preferred_element_type=f32)
                y = jnp.dot(((g * jax.nn.sigmoid(g)) * u).astype(bf16), wd_v[...], preferred_element_type=f32)
                r = jnp.sum(x8 * wr_v[...].astype(f32).reshape(1, D), axis=-1, keepdims=True)
                res_s[...] = (1.0 - gate) * (x8 + (x8 * 0.0 + y * jax.nn.sigmoid(r)))

        out_ref[...] = (gate * acc_s[...] + res_s[...])[:B].astype(out_ref.dtype)

    return kernel


def _impl(A_x, A_k_cache, A_v_cache, A_wq, A_wo, B_x, B_w_r, B_w_gate, B_w_up, B_w_down, gate_w,
          NBUF=3, KCH=(160, 4), VCH=(160, 4), WT=(8, 1792, 16), QT=(8, 2048, 4)):
    del B_x
    B, H, SK, DH = A_k_cache.shape
    D = A_x.shape[-1]
    F = B_w_gate.shape[-1]
    x2 = A_x.reshape(B, D)
    vmem = lambda a: pltpu.VMEM(a.shape, a.dtype)
    out = pl.pallas_call(
        _make_kernel(B, H, SK, DH, D, F, NBUF, KCH, VCH, WT, QT),
        out_shape=jax.ShapeDtypeStruct((B, D), A_x.dtype),
        in_specs=[pl.BlockSpec(memory_space=pl.ANY)] * 10,
        out_specs=pl.BlockSpec(memory_space=pltpu.VMEM),
        scratch_shapes=[
            vmem(x2), vmem(B_w_r), vmem(gate_w),
            vmem(A_wq), vmem(A_wo), vmem(B_w_gate), vmem(B_w_up), vmem(B_w_down),
            pltpu.VMEM((NBUF, SK, DH), A_k_cache.dtype),
            pltpu.VMEM((NBUF, SK, DH), A_v_cache.dtype),
            pltpu.VMEM((H, 8, DH), jnp.bfloat16),
            pltpu.VMEM((H, 8, DH), jnp.float32),
            pltpu.VMEM((8, D), jnp.float32),
            pltpu.VMEM((8, D), jnp.float32),
            pltpu.SemaphoreType.DMA((3,)),
            pltpu.SemaphoreType.DMA((6,)),
            pltpu.SemaphoreType.DMA((NBUF,)),
            pltpu.SemaphoreType.DMA((NBUF,)),
            pltpu.SemaphoreType.DMA((2,)),
        ],
        compiler_params=pltpu.CompilerParams(vmem_limit_bytes=100 * 1024 * 1024),
    )(x2, A_k_cache, A_v_cache, A_wq, A_wo, B_w_r, B_w_gate, B_w_up, B_w_down, gate_w)
    return out.reshape(A_x.shape)


@jax.jit
def pallas_gated_mix__mha_block_cached__moe_arch_mod__decode_kernel(
    A_x: jax.Array,
    A_k_cache: jax.Array,
    A_v_cache: jax.Array,
    A_wq: jax.Array,
    A_wo: jax.Array,
    B_x: jax.Array,
    B_w_r: jax.Array,
    B_w_gate: jax.Array,
    B_w_up: jax.Array,
    B_w_down: jax.Array,
    gate_w: jax.Array,
):
    return _impl(A_x, A_k_cache, A_v_cache, A_wq, A_wo, B_x, B_w_r, B_w_gate, B_w_up, B_w_down, gate_w)
```
